```python
import jax
import jax.numpy as jnp

def _softmax(x, axis=-1):
    return jax.nn.softmax(x, axis=axis)

def _gelu(x):
    return jax.nn.gelu(x, approximate=True)

def _silu(x):
    return jax.nn.silu(x)

def _sigmoid(x):
    return jax.nn.sigmoid(x)

def _layernorm(x, axis=-1, eps=1e-05):
    m = jnp.mean(x, axis=axis, keepdims=True)
    v = jnp.var(x, axis=axis, keepdims=True)
    return (x - m) / jnp.sqrt(v + eps)

def _scatter_add(tgt, idx, src, axis=0):
    return tgt.at[idx].add(src)

def _segment_sum(src, seg, n):
    return jax.ops.segment_sum(src, seg, n)

class _Rng:

    def __init__(self, key):
        self._k = key

    def _next(self):
        self._k, sub = jax.random.split(self._k)
        return sub

    def normal(self, shape):
        return jax.random.normal(self._next(), shape, dtype=jnp.bfloat16)

    def randint(self, lo, hi, shape):
        return jax.random.randint(self._next(), shape, lo, hi, dtype=jnp.int32)

    def uniform(self, shape, lo=0.0, hi=1.0):
        return jax.random.uniform(self._next(), shape, jnp.bfloat16, lo, hi)

    def permutation(self, n):
        return jax.random.permutation(self._next(), n)
kernel_name = 'adaLN_cond__grouped_kv_mqa__dense_activation_silu__prompt'

def _fwd_setup_inputs():
    _rng = _Rng(jax.random.key(int.from_bytes(__import__("os").urandom(4), "little")))
    _w = lambda a: (lambda t: t.astype(jnp.bfloat16) if jnp.issubdtype(t.dtype, jnp.floating) else t)(jnp.asarray(a))

    def _A_setup():
        B, S, D, H = (1, 2048, 640, 32)
        Dh = D // H
        return {'x': _w((lambda *s: _rng.normal(s) * 0.05)(B, S, D)), 'wq': _w((lambda *s: _rng.normal(s) * 0.05)(D, H * Dh)), 'wk': _w((lambda *s: _rng.normal(s) * 0.05)(D, Dh)), 'wv': _w((lambda *s: _rng.normal(s) * 0.05)(D, Dh)), 'wo': _w((lambda *s: _rng.normal(s) * 0.05)(H * Dh, D))}
    _A_in = _A_setup()

    def _B_setup():
        B, S, D, F = (1, 2048, 640, 1728)
        return {'x': _w((lambda *s: _rng.normal(s) * 0.05)(B, S, D)), 'w1': _w((lambda *s: _rng.normal(s) * 0.05)(D, F) * D ** (-0.5)), 'w2': _w((lambda *s: _rng.normal(s) * 0.05)(F, D) * F ** (-0.5))}
    _B_in = _B_setup()
    return {'A_x': _A_in['x'], 'A_wq': _A_in['wq'], 'A_wk': _A_in['wk'], 'A_wv': _A_in['wv'], 'A_wo': _A_in['wo'], 'B_x': _B_in['x'], 'B_w1': _B_in['w1'], 'B_w2': _B_in['w2'], 'c': _w((lambda *s: _rng.normal(s) * 0.05)(1, 640)), 'w_mod': _w((lambda *s: _rng.normal(s) * 0.05)(640, 6 * 640) * 640 ** (-0.5))}

def _fwd_reference(A_x, A_wq, A_wk, A_wv, A_wo, B_x, B_w1, B_w2, c, w_mod):

    def _A_ref(x, wq, wk, wv, wo):
        B, S, D = x.shape
        H = 32
        Dh = D // H
        q = (lambda x, *d: x.transpose(*d))((x @ wq).reshape(B, S, H, Dh), 0, 2, 1, 3)
        k = x @ wk
        v = x @ wv
        scores = jnp.einsum('bhqd,bkd->bhqk', q, k) * Dh ** (-0.5)
        p = _softmax(scores, axis=-1)
        o = jnp.einsum('bhqk,bkd->bhqd', p, v)
        return (lambda x, *d: x.transpose(*d))(o, 0, 2, 1, 3).reshape(B, S, H * Dh) @ wo

    def _B_ref(x, w1, w2):
        h = jnp.einsum('bsd,df->bsf', x, w1)
        h = _silu(h)
        out = jnp.einsum('bsf,fd->bsd', h, w2)
        return out
    x = A_x
    mod = (_silu(c) @ w_mod).reshape(c.shape[0], 6, 1, -1)
    sa, ca, ga, sb, cb, gb = (mod[:, 0].copy(), mod[:, 1].copy(), mod[:, 2].copy(), mod[:, 3].copy(), mod[:, 4].copy(), mod[:, 5].copy())
    h = _layernorm(x, axis=-1) * (1 + ca) + sa
    x = x + ga * _A_ref(h, A_wq, A_wk, A_wv, A_wo)
    h = _layernorm(x, axis=-1) * (1 + cb) + sb
    x = x + gb * _B_ref(h, B_w1, B_w2)
    return x

def setup_inputs():
    _inp = _fwd_setup_inputs()
    _gk = jax.random.fold_in(jax.random.key(int.from_bytes(__import__("os").urandom(4), "little")), 2 ** 31 - 1)
    _shapes = [[1, 2048, 640]]
    _dtypes = ['bfloat16']
    _gks = jax.random.split(_gk, len(_shapes))
    _gs = [jax.random.normal(k, s, dtype=jnp.dtype(d)) * 0.05 for k, s, d in zip(_gks, _shapes, _dtypes)]
    _inp['grad_out'] = _gs[0]
    return _inp

def reference(A_x, A_wq, A_wk, A_wv, A_wo, B_w1, B_w2, c, w_mod, B_x, grad_out):
    _const = dict(B_x=B_x)

    def _f(*_d):
        return _fwd_reference(**{'A_x': _d[0], 'A_wq': _d[1], 'A_wk': _d[2], 'A_wv': _d[3], 'A_wo': _d[4], 'B_w1': _d[5], 'B_w2': _d[6], 'c': _d[7], 'w_mod': _d[8], **_const})
    _out, _vjp = jax.vjp(_f, A_x, A_wq, A_wk, A_wv, A_wo, B_w1, B_w2, c, w_mod)
    _grads = _vjp(grad_out)
    _out0 = jnp.asarray(_out)
    return (_out0, *[jnp.asarray(_g) for _g in _grads])
```

```python
import math

import jax
import jax.numpy as jnp
from jax import lax
import jax.experimental.pallas as pl
import jax.experimental.pallas.tpu as pltpu

F32 = jnp.float32
BF16 = jnp.bfloat16
_NN = (((1,), (0,)), ((), ()))
_NT = (((1,), (1,)), ((), ()))

HEADS = 32
HP = 24
BQ = 256
NC = 2 * BQ
CK = 128
TC = 512
EPS = 1e-5


def _dot(a, b, dims=_NN):
    return lax.dot_general(a, b, dims, preferred_element_type=F32)


def _round(x):
    return x.astype(BF16).astype(F32)


def _lanes(v, n):
    return jnp.concatenate([v] * (n // 128), axis=1)


def _fold(v):
    out = v[:, :128]
    for j in range(1, v.shape[1] // 128):
        out = out + v[:, j * 128:(j + 1) * 128]
    return out


def _normalize(x):
    inv_d = 1.0 / x.shape[0]
    xc = x - jnp.sum(x, axis=0, keepdims=True) * inv_d
    rstd = lax.rsqrt(jnp.sum(xc * xc, axis=0, keepdims=True) * inv_d + EPS)
    return xc * rstd, rstd


def _normalize_bwd(dxh, xh, rstd):
    inv_d = 1.0 / xh.shape[0]
    m1 = jnp.sum(dxh, axis=0, keepdims=True) * inv_d
    m2 = jnp.sum(dxh * xh, axis=0, keepdims=True) * inv_d
    return rstd * (dxh - m1 - xh * m2)


def _kernel(
    x_hbm, wq_hbm, wkt_hbm, wvt_hbm, wo_hbm, w1t_hbm, w2_hbm, c_hbm, wm_hbm, g_hbm,
    out_hbm, dx_hbm, gwq_hbm, gwkt_hbm, gwvt_hbm, gwo_hbm, gw1t_hbm, gw2_hbm, gc_hbm, gwm_hbm,
    xs, gs, wq, wkt, wvt, wo, w1t, w2, cb, wm,
    wqkv_t, wkv, wot, w1, w2t,
    xt, qbuf, kp, vp, kt, vt, dkt, dvt,
    pbuf, sbuf, obuf, dobuf, dx1,
    modc, sct, dmod, gc_acc,
    dw1t, dw2, dwo, act_s, du_s, h_s, dq_s,
    sem_in, sem_out,
):
    S, D = xs.shape
    FF = w2.shape[0]
    DH = D // HEADS
    NB = S // BQ
    U = HEADS // 2
    NCH = S // CK
    NT = S // TC
    scale = DH ** -0.5
    log2e = math.log2(math.e)

    row8 = lax.broadcasted_iota(jnp.int32, (8, BQ), 0)
    row24 = lax.broadcasted_iota(jnp.int32, (HP, NC), 0)

    def split_pair(v, u):
        even = v[2 * DH * u:2 * DH * u + HP]
        odd = pltpu.roll(v[2 * DH * u + 16:2 * DH * u + 16 + HP], HP - 4, 0)
        return jnp.concatenate([even, odd], axis=1)

    def merge_pair(w):
        even = w[:, :BQ]
        odd = pltpu.roll(w[:, BQ:], 4, 0)
        mid = jnp.where(row8 < 4, even[16:24], odd[0:8])
        return jnp.concatenate([even[0:16], mid, odd[8:24]], axis=0)

    def weights32(w):
        return jnp.concatenate([w, jnp.zeros((32 - HP, NC), F32)], axis=0).astype(BF16)

    def cin(i, src, dst):
        return pltpu.make_async_copy(src, dst, sem_in.at[i])

    def cout(i, src, dst):
        return pltpu.make_async_copy(src, dst, sem_out.at[i])

    cp_c = cin(0, c_hbm, cb)
    cp_wm0 = cin(1, wm_hbm.at[:, pl.ds(0, 2 * D)], wm.at[:, pl.ds(0, 2 * D)])
    cp_wq = cin(2, wq_hbm, wq)
    cp_wk = cin(3, wkt_hbm, wkt)
    cp_wv = cin(4, wvt_hbm, wvt)
    cp_wm1 = cin(5, wm_hbm.at[:, pl.ds(2 * D, 4 * D)], wm.at[:, pl.ds(2 * D, 4 * D)])
    cp_wo = cin(6, wo_hbm, wo)
    cp_w1 = cin(7, w1t_hbm, w1t)
    cp_w2 = cin(8, w2_hbm, w2)
    cp_g = cin(9, g_hbm, gs)
    cp_x = [cin(10 + t, x_hbm.at[pl.ds(t * TC, TC)], xs.at[pl.ds(t * TC, TC)]) for t in range(NT)]
    for cp in (cp_c, cp_wq, cp_wk, cp_wv, cp_x[0], cp_wm0):
        cp.start()

    dkt[...] = jnp.zeros_like(dkt)
    dvt[...] = jnp.zeros_like(dvt)
    dmod[...] = jnp.zeros_like(dmod)
    dw1t[...] = jnp.zeros_like(dw1t)
    dw2[...] = jnp.zeros_like(dw2)
    dwo[...] = jnp.zeros_like(dwo)

    cp_c.wait()
    cf = cb[...].astype(F32)
    c_sig = jax.nn.sigmoid(cf)
    sc = _round(cf * c_sig)
    sct[...] = jnp.broadcast_to(sc, (128, D)).T
    sc8 = jnp.broadcast_to(sc, (8, D))

    def modulation(parts):
        for j in parts:
            m = _dot(sc8, wm[:, j * D:(j + 1) * D])
            if j in (1, 4):
                m = m + 1.0
            modc[j] = jnp.broadcast_to(m[0:1], (128, D)).T

    cp_wq.wait()
    cp_wk.wait()
    cp_wv.wait()
    zpad = jnp.zeros((32 - DH, D), F32)
    kv_rows = jnp.concatenate([wkt[...].astype(F32), zpad, wvt[...].astype(F32), zpad], axis=0)
    wqkv_t[0:D] = wq[...].T
    wqkv_t[D:D + 64] = kv_rows.astype(BF16)
    wkv[...] = jnp.concatenate([kv_rows, jnp.zeros((64, D), F32)], axis=0).T.astype(BF16)

    cp_wm0.wait()
    for cp in cp_x[1:]:
        cp.start()
    modulation((0, 1))

    rowt = lax.broadcasted_iota(jnp.int32, (32, TC), 0)
    for t in range(NT):
        cp_x[t].wait()
        if t == 1:
            for cp in (cp_wo, cp_wm1, cp_w1, cp_w2, cp_g):
                cp.start()
        cols = slice(t * TC, (t + 1) * TC)
        xb = xs[cols].T
        for j in range(TC // BQ):
            xt[t * (TC // BQ) + j] = xb[:, j * BQ:(j + 1) * BQ]
        xh, _ = _normalize(xb.astype(F32))
        h = (xh * _lanes(modc[1], TC) + _lanes(modc[0], TC)).astype(BF16)
        qkv = _dot(wqkv_t[...], h)
        q = _round(qkv[0:D] * (scale * log2e))
        for j in range(TC // BQ):
            qj = q[:, j * BQ:(j + 1) * BQ]
            for u in range(U):
                qbuf[(t * (TC // BQ) + j) * U + u] = jnp.where(row24 < DH, split_pair(qj, u), 0.0)
        k = _round(qkv[D:D + 32])
        v = _round(qkv[D + 32:D + 64])
        kt[:, cols] = k[0:HP]
        vt[:, cols] = jnp.where(rowt == DH, 1.0, v)[0:HP]
        neg = jnp.where((rowt == DH) | (rowt == DH + 1), -1.0, v)
        zrows = jnp.zeros((96, TC), F32)
        kp[cols] = jnp.concatenate([k, zrows], axis=0).T[:, 0:32].astype(BF16)
        vp[cols] = jnp.concatenate([neg, zrows], axis=0).T[:, 0:32].astype(BF16)

    cp_wo.wait()
    wot[...] = wo[...].T
    cp_wm1.wait()
    modulation((2, 3, 4, 5))
    cp_w1.wait()
    w1[...] = w1t[...].T
    cp_w2.wait()
    w2t[...] = w2[...].T
    cp_g.wait()

    def keys(c):
        return slice(c * CK, (c + 1) * CK)

    def pkeys(c):
        return slice(c * CK // 2, (c + 1) * CK // 2)

    def fwd_step(u_old, m_old, g_new):
        if g_new is not None:
            qw = weights32(qbuf[g_new])
            m_new = None
        acc = None
        for c in range(NCH):
            if u_old is not None:
                p = jnp.exp2(sbuf[keys(c)] - m_old).astype(BF16)
                pbuf[u_old, pkeys(c)] = pltpu.bitcast(p, jnp.uint32)
            if g_new is not None:
                s = _dot(kp[keys(c)], qw)
            if u_old is not None:
                pv = _dot(vt[:, keys(c)], p)
                acc = pv if acc is None else acc + pv
            if g_new is not None:
                sbuf[keys(c)] = s
                mc = jnp.max(s.reshape(CK // 8, 8, NC), axis=0)
                m_new = mc if m_new is None else jnp.maximum(m_new, mc)
        if u_old is not None:
            linv = 1.0 / acc[DH:DH + 1]
            obuf[u_old] = jnp.where(row24 == DH, linv, acc * linv)
        if g_new is not None:
            return jnp.max(m_new, axis=0, keepdims=True)
        return None

    def bwd_steps(units, base):
        pending = None
        accs = {}

        def tail(i, u, c, p, ds, dow, qf):
            dvt[:, keys(c)] += _dot(dow, p, _NT)
            dkt[:, keys(c)] += _dot(qf, ds, _NT)
            dq = _dot(kt[:, keys(c)], ds)
            accs[i] = dq if c == 0 else accs[i] + dq
            if c == NCH - 1:
                qbuf[base + u] = accs[i]

        for i, u in enumerate(units):
            dow = dobuf[u]
            qf = qbuf[base + u]
            dw = weights32(dow)
            for c in range(NCH):
                dp = _dot(vp[keys(c)], dw)
                if pending is not None:
                    tail(*pending)
                p = pltpu.bitcast(pbuf[u, pkeys(c)], BF16)
                ds = (p.astype(F32) * dp).astype(BF16)
                pending = (i, u, c, p, ds, dow, qf)
        tail(*pending)

    def dense(b):
        rows = pl.ds(pl.multiple_of(b * BQ, BQ), BQ)
        ga, sb, cb1, gb = (_lanes(modc[j], BQ) for j in (2, 3, 4, 5))
        g = gs[rows].T.astype(F32)
        df = (g * gb).astype(BF16)
        o = jnp.concatenate([merge_pair(obuf[u]) for u in range(U)], axis=0).astype(BF16)
        a = _dot(wot[...], o)
        dact = _dot(w2[...], df)
        x1 = xt[b].astype(F32) + ga * a
        xh2, rstd2 = _normalize(x1)
        h2 = (xh2 * cb1 + sb).astype(BF16)
        uu = _dot(w1t[...], h2)
        sig = jax.nn.sigmoid(uu)
        act = uu * sig
        act_s[...] = act.astype(BF16)
        du_s[...] = (dact * (sig + act * (1.0 - sig))).astype(BF16)
        dw2[...] += _dot(act_s[...], df, _NT)
        dh2 = _dot(w1[...], du_s[...])
        f = _dot(w2t[...], act_s[...])
        d1 = g + _normalize_bwd(dh2 * cb1, xh2, rstd2)
        dx1[b] = d1
        da = (d1 * ga).astype(BF16)
        do = _dot(wo[...], da)
        dw1t[...] += _dot(du_s[...], h2, _NT)
        dwo[...] += _dot(o, da, _NT)
        gs[rows] = (x1 + gb * f).astype(BF16).T
        dmod[2] += _fold(d1 * a)
        dmod[3] += _fold(dh2)
        dmod[4] += _fold(dh2 * xh2)
        dmod[5] += _fold(g * f)
        for u in range(U):
            ou = obuf[u]
            dos = jnp.where(row24 < DH, _round(split_pair(do, u) * ou[DH:DH + 1]), 0.0)
            delta = jnp.sum(dos * ou, axis=0, keepdims=True)
            hi = _round(delta)
            dobuf[u] = jnp.where(row24 == DH, hi, jnp.where(row24 == DH + 1, _round(delta - hi), dos))

    def modulation_bwd(parts):
        total = None
        for j in parts:
            drow = jnp.sum(dmod[j].T, axis=0, keepdims=True)
            cols = slice(j * D, (j + 1) * D)
            part = _fold(wm[:, cols].astype(F32) * drow)
            total = part if total is None else total + part
            wm[:, cols] = (_lanes(sct[...], D) * drow).astype(BF16)
        return total

    cp_gw1 = cout(0, w1t, gw1t_hbm)
    cp_gw2 = cout(1, w2, gw2_hbm)
    cp_gwo = cout(2, wo, gwo_hbm)
    cp_gwm1 = cout(3, wm.at[:, pl.ds(2 * D, 4 * D)], gwm_hbm.at[:, pl.ds(2 * D, 4 * D)])
    cp_out = cout(4, gs, out_hbm)

    def block(b, carry):
        base = b * U
        m = fwd_step(None, None, base)
        m = fwd_step(0, m, base + 1)

        def fwd_body(i, m):
            m = fwd_step(2 * i + 1, m, base + 2 * i + 2)
            return fwd_step(2 * i + 2, m, base + 2 * i + 3)

        m = lax.fori_loop(0, U // 2 - 1, fwd_body, m)
        fwd_step(U - 1, m, None)
        dense(b)

        def bwd_body(i, carry):
            bwd_steps((2 * i, 2 * i + 1), base)
            return carry

        lax.fori_loop(0, U // 2, bwd_body, 0)
        return carry

    lax.fori_loop(0, NB, block, 0)

    cp_out.start()
    w1t[...] = dw1t[...].astype(BF16)
    cp_gw1.start()
    w2[...] = dw2[...].astype(BF16)
    cp_gw2.start()
    wo[...] = dwo[...].astype(BF16)
    cp_gwo.start()
    gc_acc[...] = modulation_bwd((2, 3, 4, 5))
    cp_gwm1.start()

    rowh = lax.broadcasted_iota(jnp.int32, (HP, TC), 0)
    cp_dx = [cout(10 + t, xs.at[pl.ds(t * TC, TC)], dx_hbm.at[pl.ds(t * TC, TC)]) for t in range(NT)]
    for t in range(NT):
        cols = slice(t * TC, (t + 1) * TC)
        blocks = range(t * (TC // BQ), (t + 1) * (TC // BQ))
        dq = jnp.concatenate(
            [jnp.concatenate([merge_pair(qbuf[b * U + u]) for u in range(U)], axis=0) for b in blocks],
            axis=1)
        dq = (dq * scale).astype(BF16)
        z8 = jnp.zeros((8, TC), F32)
        dkv = jnp.concatenate(
            [dkt[:, cols] * (1.0 / log2e), z8, jnp.where(rowh < DH, dvt[:, cols], 0.0), z8],
            axis=0).astype(BF16)
        dq_s[0:D, cols] = dq
        dq_s[D:D + 64, cols] = dkv
        dh = _dot(wq[...], dq) + _dot(wkv[:, 0:64], dkv)
        xh, rstd = _normalize(jnp.concatenate([xt[b] for b in blocks], axis=1).astype(F32))
        ca1 = _lanes(modc[1], TC)
        h_s[:, cols] = (xh * ca1 + _lanes(modc[0], TC)).astype(BF16)
        dmod[0] += _fold(dh)
        dmod[1] += _fold(dh * xh)
        d0 = jnp.concatenate([dx1[b] for b in blocks], axis=1) + _normalize_bwd(dh * ca1, xh, rstd)
        xs[cols] = d0.astype(BF16).T
        cp_dx[t].start()

    gc_col = gc_acc[...] + modulation_bwd((0, 1))
    cp_gwm0 = cout(5, wm.at[:, pl.ds(0, 2 * D)], gwm_hbm.at[:, pl.ds(0, 2 * D)])
    cp_gwm0.start()
    gsc = jnp.sum(gc_col.T, axis=0, keepdims=True)
    cb[...] = (gsc * c_sig * (1.0 + cf * (1.0 - c_sig))).astype(BF16)
    cp_gc = cout(6, cb, gc_hbm)
    cp_gc.start()

    gkv = _dot(dq_s[D:D + 64], h_s[...], _NT)
    wkt[...] = gkv[0:DH].astype(BF16)
    wvt[...] = gkv[32:32 + DH].astype(BF16)
    cp_gwk = cout(7, wkt, gwkt_hbm)
    cp_gwv = cout(8, wvt, gwvt_hbm)
    cp_gwk.start()
    cp_gwv.start()
    wot[...] = _dot(h_s[...], dq_s[0:D], _NT).astype(BF16)
    cp_gwq = cout(9, wot, gwq_hbm)
    cp_gwq.start()

    for cp in (cp_out, cp_gw1, cp_gw2, cp_gwo, cp_gwm1, *cp_dx, cp_gwm0, cp_gc, cp_gwk, cp_gwv, cp_gwq):
        cp.wait()


@jax.jit
def pallas_adaLN_cond__grouped_kv_mqa__dense_activation_silu__prompt_kernel(
    A_x: jax.Array,
    A_wq: jax.Array,
    A_wk: jax.Array,
    A_wv: jax.Array,
    A_wo: jax.Array,
    B_x: jax.Array,
    B_w1: jax.Array,
    B_w2: jax.Array,
    c: jax.Array,
    w_mod: jax.Array,
    grad_out: jax.Array,
):
    del B_x
    _, S, D = A_x.shape
    FF = B_w1.shape[1]
    DH = D // HEADS
    NB = S // BQ
    U = HEADS // 2
    vmem = pltpu.VMEM

    def sds(*shape):
        return jax.ShapeDtypeStruct(shape, BF16)

    scratch = [
        vmem((S, D), BF16), vmem((S, D), BF16), vmem((D, D), BF16), vmem((DH, D), BF16),
        vmem((DH, D), BF16), vmem((D, D), BF16), vmem((FF, D), BF16), vmem((FF, D), BF16),
        vmem((1, D), BF16), vmem((D, 6 * D), BF16),
        vmem((D + 64, D), BF16), vmem((D, 128), BF16), vmem((D, D), BF16),
        vmem((D, FF), BF16), vmem((D, FF), BF16),
        vmem((NB, D, BQ), BF16), vmem((NB * U, HP, NC), F32),
        vmem((S, 32), BF16), vmem((S, 32), BF16),
        vmem((HP, S), F32), vmem((HP, S), F32), vmem((HP, S), F32), vmem((HP, S), F32),
        vmem((U, S // 2, NC), jnp.uint32), vmem((S, NC), F32),
        vmem((U, HP, NC), F32), vmem((U, HP, NC), F32), vmem((NB, D, BQ), F32),
        vmem((6, D, 128), F32), vmem((D, 128), F32), vmem((6, D, 128), F32), vmem((D, 128), F32),
        vmem((FF, D), F32), vmem((FF, D), F32), vmem((D, D), F32),
        vmem((FF, BQ), BF16), vmem((FF, BQ), BF16), vmem((D, S), BF16), vmem((D + 64, S), BF16),
        pltpu.SemaphoreType.DMA((10 + S // TC,)), pltpu.SemaphoreType.DMA((10 + S // TC,)),
    ]
    hbm = pl.BlockSpec(memory_space=pl.ANY)
    out, dx, gwq, gwkt, gwvt, gwo, gw1t, gw2, gc, gwm = pl.pallas_call(
        _kernel,
        in_specs=[hbm] * 10,
        out_specs=[hbm] * 10,
        out_shape=[sds(S, D), sds(S, D), sds(D, D), sds(DH, D), sds(DH, D), sds(D, D),
                   sds(FF, D), sds(FF, D), sds(1, D), sds(D, 6 * D)],
        scratch_shapes=scratch,
        compiler_params=pltpu.CompilerParams(vmem_limit_bytes=120 * 1024 * 1024),
    )(A_x.reshape(S, D), A_wq, A_wk.T, A_wv.T, A_wo, B_w1.T, B_w2, c, w_mod, grad_out.reshape(S, D))
    return (out.reshape(1, S, D), dx.reshape(1, S, D), gwq, gwkt.T, gwvt.T, gwo, gw1t.T, gw2, gc, gwm)
```

```python
import math

import jax
import jax.numpy as jnp
from jax import lax
import jax.experimental.pallas as pl
import jax.experimental.pallas.tpu as pltpu

F32 = jnp.float32
BF16 = jnp.bfloat16
U32 = jnp.uint32
_NN = (((1,), (0,)), ((), ()))
_NT = (((1,), (1,)), ((), ()))

HEADS = 32
EPS = 1e-5
SAFE_LOG2 = 56.0

HP = 24
KV = 2 * HP
BQ = 256
NC = 2 * BQ
CK = 128
NV, NF, ND = 32, 16, 16
KH = 256
FM = 432

SCHED_FWD = ("S0P3", [NF] * 23 + [0] * 9, [4] * 32)
SCHED_MERGED = ("D0K1V0P1S0Q0", [NV] * 31 + [24], [2] * 16 + [3] + [2] * 14 + [4])
SCHED_BWD = ("D0V0K1Q1", [0] + [ND] * 31, [0] * 32)


def _dot(a, b, dims=_NN):
    return lax.dot_general(a, b, dims, preferred_element_type=F32)


def _round(x):
    return x.astype(BF16).astype(F32)


def _words(x):
    return pltpu.bitcast(x, U32)


def _bf16(w):
    return pltpu.bitcast(w, BF16)


def _even_odd(w):
    return pltpu.bitcast(w << 16, F32), pltpu.bitcast(w & jnp.uint32(0xFFFF0000), F32)


def _interleave(even, odd):
    return (even >> 16) | (odd & jnp.uint32(0xFFFF0000))


def _half(r):
    return slice(r.start // 2, r.stop // 2)


def _lanes(v, n):
    return jnp.concatenate([v] * (n // 128), axis=1)


def _fold(v):
    out = v[:, :128]
    for j in range(128, v.shape[1], 128):
        out = out + v[:, j:j + 128]
    return out


def _after(seed, value, prev):
    keep = lax.broadcasted_iota(jnp.int32, value.shape, 0) > -1 - seed
    return jnp.where(keep, value, prev)


def _paced(seed, fn, stat, rows, step):
    stat = jnp.broadcast_to(stat, (8, stat.shape[1]))
    out = []
    for r in range(0, rows, step):
        if out:
            stat = _after(seed, stat, out[-1][-8:])
        out.append(fn(slice(r, r + step), jnp.concatenate([stat] * (step // 8), axis=0)))
    return jnp.concatenate(out, axis=0)


def _row_mean(x):
    return jnp.sum(x, axis=0, keepdims=True) * (1.0 / x.shape[0])


def _center(seed, x):
    tiles = []
    for t in range(0, x.shape[1], 128):
        xl = x[:, t:t + 128]
        if tiles:
            xl = jnp.concatenate([_after(seed, xl[:8], tiles[-1][2]), xl[8:]], axis=0)
        mean = _row_mean(xl)
        xc = xl - mean
        tiles.append((xc, mean, lax.rsqrt(_row_mean(xc * xc) + EPS)))
    return [jnp.concatenate(parts, axis=1) for parts in zip(*tiles)]


def _left_terms(x11, x12, x21, x22):
    return [t.astype(BF16) for t in (x11 + x22, x21 + x22, x11, x22, x11 + x12, x21 - x11, x12 - x22)]


def _left_words(*words):
    parity = list(zip(*[_even_odd(w) for w in words]))

    def combine(op, i, j):
        return _interleave(*[pltpu.bitcast(op(x[i], x[j]), U32) + jnp.uint32(0x8000) for x in parity])

    return [combine(jnp.add, 0, 3), combine(jnp.add, 2, 3), words[0], words[3],
            combine(jnp.add, 0, 1), combine(jnp.subtract, 2, 0), combine(jnp.subtract, 1, 3)]


def _right_order(left):
    return [left[j] for j in (0, 2, 6, 5, 3, 4, 1)]


def _strassen(left, right, dims=_NN):
    m2, m4, m3, m5, m1, m7, m6 = (_dot(left[j], right[j], dims) for j in (1, 3, 2, 4, 0, 6, 5))
    return m4 - m5 + m1 + m7, m3 + m5, m2 + m4, m3 - m2 + m1 + m6


def _kernel(
    x_hbm, wq_hbm, wkt_hbm, wvt_hbm, wo_hbm, w1t_hbm, w2_hbm, c_hbm, wm_hbm, g_hbm,
    out_hbm, dx_hbm, gwq_hbm, gwkt_hbm, gwvt_hbm, gwo_hbm, gw1t_hbm, gw2_hbm, gc_hbm, gwm_hbm,
    *,
    pbuf, carry_o, carry_dq, carry_ds, obuf, omrg, dobuf, qbuf, kp, vp, kt, vt, dkt, dvt,
    ktab, kvtab, qrow, xs, gs, wq, wo, wf, wm, wqkv, wot, wf_terms, wft_terms, xt, ht, dx1,
    dq_rest, stats, modc, sct, dmod, gc_col, dwf, dwo, ffn_terms, wqkv_t, drow, wkt, wvt, cb,
    sem_in, sem_out,
):
    S, D = xs.shape
    FF = dwf.shape[1]
    FH = FF // 2
    FT = wft_terms.shape[2]
    DH = D // HEADS
    NB = S // BQ
    U = HEADS // 2
    NCH = S // CK
    CPB = BQ // CK
    QE = D - dq_rest.shape[1]
    scale = DH ** -0.5
    log2e = math.log2(math.e)

    row8 = lax.broadcasted_iota(jnp.int32, (8, BQ), 0)
    rowb = lax.broadcasted_iota(jnp.int32, (HP, BQ), 0)
    rowc = lax.broadcasted_iota(jnp.int32, (HP, NC), 0)

    def split_pair(v, u):
        even = v[2 * DH * u:2 * DH * u + HP]
        odd = pltpu.roll(v[2 * DH * u + 16:2 * DH * u + 16 + HP], HP - 4, 0)
        return jnp.concatenate([even, odd], axis=1)

    def merge_pair(w):
        even = w[:, :BQ]
        odd = pltpu.roll(w[:, BQ:], 4, 0)
        mid = jnp.where(row8 < 4, even[16:24], odd[0:8])
        return jnp.concatenate([even[0:16], mid, odd[8:24]], axis=0)

    def aligned(start, size, align):
        return pl.ds(start if isinstance(start, int) else pl.multiple_of(start, align), size)

    def block_rows(b):
        return aligned(b * BQ, BQ, BQ)

    def slab(i):
        return aligned(i * 128, 128, 128)

    def share(u, total):
        size = pl.cdiv(total, 8 * U) * 16
        return aligned(jnp.minimum(u * size, total - size), size, 16)

    def side_by_side(ref):
        return jnp.concatenate([ref[j] for j in range(ref.shape[0])], axis=1)

    def mod(j, rows=slice(None)):
        return _lanes(modc[j, rows], BQ)

    def cin(i, src, dst):
        return pltpu.make_async_copy(src, dst, sem_in.at[i])

    def cout(i, src, dst):
        return pltpu.make_async_copy(src, dst, sem_out.at[i])

    def cp_x(b):
        return cin(10 + b, x_hbm.at[block_rows(b)], xs.at[block_rows(b)])

    norm1_cols, other_cols = pl.ds(0, 2 * D), pl.ds(2 * D, 4 * D)
    cp_c = cin(0, c_hbm, cb)
    cp_wm0 = cin(1, wm_hbm.at[:, norm1_cols], wm.at[:, norm1_cols])
    cp_wq = cin(2, wq_hbm, wq)
    cp_wk = cin(3, wkt_hbm, wkt)
    cp_wv = cin(4, wvt_hbm, wvt)
    cp_wm1 = cin(5, wm_hbm.at[:, other_cols], wm.at[:, other_cols])
    cp_wo = cin(6, wo_hbm, wo)
    cp_w1 = cin(7, w1t_hbm, wf.at[0, pl.ds(0, FF)])
    cp_w2 = cin(8, w2_hbm, wf.at[1, pl.ds(0, FF)])
    cp_g = cin(9, g_hbm, gs)
    for cp in (cp_c, cp_wq, cp_wk, cp_wv, cp_x(0), cp_wm0, cp_x(1)):
        cp.start()

    def zero_slab(i, carry):
        dwo[slab(i)] = jnp.zeros((128, D), F32)
        dmod[:, slab(i)] = jnp.zeros((6, 128, 128), F32)
        return carry

    lax.fori_loop(0, D // 128, zero_slab, 0)
    qbuf[0] = jnp.zeros((HP, NC), F32)
    carry_o[...] = jnp.ones_like(carry_o)
    carry_dq[...] = jnp.zeros_like(carry_dq)
    carry_ds[...] = jnp.zeros_like(carry_ds)
    pbuf[U - 1, (S - 3 * CK) // 2:] = jnp.zeros((3 * CK // 2, NC), U32)
    wf[:, FF:] = jnp.zeros((2, wf.shape[1] - FF, D), BF16)

    cp_c.wait()
    cf = cb[...].astype(F32)
    c_sig = jax.nn.sigmoid(cf)
    sc = _round(cf * c_sig)
    sct[...] = jnp.broadcast_to(sc, (128, D)).T

    def modulation(j):
        m = _dot(jnp.broadcast_to(sc, (8, D)), wm[:, j * D:(j + 1) * D])
        if j % 3 == 1:
            m = m + 1.0
        modc[j] = jnp.broadcast_to(m[0:1], (128, D)).T

    def zero_weight_grad(w):
        def body(i, carry):
            dwf[w, aligned(i * 64, 64, 64)] = jnp.zeros((64, D), F32)
            return carry

        lax.fori_loop(0, FF // 64, body, 0)

    zero_weight_grad(0)
    cp_wq.wait()
    cp_wk.wait()
    cp_wv.wait()
    zpad = jnp.zeros((HP - DH, D), F32)
    kv_rows = jnp.concatenate([wkt[...].astype(F32), zpad, wvt[...].astype(F32), zpad], axis=0)
    wqkv_t[0:KV // 2] = _words(kv_rows.astype(BF16))
    wqkv_t[KV // 2:(KV + D) // 2] = _words(wq[...].T)
    wqkv[:, :D] = _words(wq[...])
    wqkv[:, D:] = _words(jnp.concatenate([kv_rows, jnp.zeros((128 - KV, D), F32)], axis=0).astype(BF16).T)

    def norm1(b):
        xb = xs[block_rows(b)].T
        xt[b] = _words(xb)
        xc, mean, rstd = _center(b, xb.astype(F32))
        stats[b] = jnp.where(row8 == 0, mean, rstd)
        return xc, rstd

    def modulate(b, xc, rstd, step):
        h = _paced(b, lambda r, rs: xc[r] * rs * mod(1, r) + mod(0, r), rstd, D, step)
        ht[b] = _words(h.astype(BF16))

    def column_table(ref, c, rows):
        for d in range(DH):
            col = jnp.broadcast_to(rows[:, d:d + 1], (rows.shape[0], 128))
            for r in range(rows.shape[0] // 8):
                ref[c, r, d] = col[8 * r:8 * r + 8]

    def project(b, norms):
        q_sq, k_sq = norms

        @pl.when(b + 1 < NB)
        def _():
            cp_x(b + 1).wait()

        qkv = _dot(_bf16(wqkv_t[0:(KV + D) // 2]), _bf16(ht[b]))
        nxt = jnp.minimum(b + 1, NB - 1)
        modulate(nxt, *norm1(nxt), 16)
        for u in range(U):
            qu = split_pair(qkv[KV:], u)
            qu = jnp.concatenate([qu[:16], jnp.where(rowc[16:] < DH, qu[16:], 0.0)], axis=0)
            qbuf[b * U + u + 1] = qu
            sq = qu * qu
            q_sq = jnp.maximum(q_sq, sq[0:8] + sq[8:16] + sq[16:24])
        k = _round(qkv[0:HP] * (scale * log2e))
        v = _round(qkv[HP:KV])
        k_sq = jnp.maximum(k_sq, jnp.sum(k * k, axis=0, keepdims=True))
        kt[b] = _round(qkv[0:HP] * scale)
        vt[b] = jnp.where(rowb == DH, 1.0, v)
        dkt[b] = jnp.zeros((HP, BQ), F32)
        dvt[b] = jnp.zeros((HP, BQ), F32)
        zrows = jnp.zeros((128 - HP, BQ), F32)
        vneg = jnp.where((rowb >= DH) & (rowb < DH + 2), -1.0, v)
        kneg = jnp.where((rowb >= DH) & (rowb < DH + 3), -1.0, k)
        vp[block_rows(b)] = jnp.concatenate([vneg, zrows], axis=0).T[:, 0:HP]
        parity = _even_odd(_words(jnp.concatenate([kneg, zrows], axis=0).astype(BF16).T))
        krows = jnp.concatenate([part[r:r + 8] for r in range(0, BQ // 2, 8) for part in parity], axis=0)
        kp[block_rows(b)] = krows[:, 0:HP]
        for j in range(CPB):
            column_table(ktab, b * CPB + j, krows[(j + 1) * CK - NF:(j + 1) * CK])
        return q_sq, k_sq

    cp_x(0).wait()
    omrg[...], rstd0 = norm1(0)
    zero_weight_grad(1)
    cp_wm0.wait()
    for cp in [cp_x(b) for b in range(2, NB)] + [cp_wo, cp_w1, cp_w2]:
        cp.start()
    modulation(0)
    modulation(1)
    modulate(0, omrg[...], rstd0, D)
    q_sq, k_sq = lax.fori_loop(0, NB, project, (jnp.zeros((8, NC), F32), jnp.zeros((1, BQ), F32)))

    bound_sq = jnp.max(jnp.sum(q_sq, axis=0, keepdims=True)) * jnp.max(k_sq)

    @pl.when(jnp.logical_not(bound_sq <= SAFE_LOG2 * SAFE_LOG2))
    def _():
        def true_max(g, carry):
            qu = _round(qbuf[g])
            qbuf[g] = qu

            def chunk_max(c, m):
                return jnp.maximum(m, jnp.max(_dot(kp[slab(c)], qbuf[g]), axis=0, keepdims=True))

            m = lax.fori_loop(0, S // 128, chunk_max, jnp.full((1, NC), -jnp.inf, F32))
            hi = _round(m)
            mid = _round(m - hi)
            for r, piece in enumerate((hi, mid, m - hi - mid, -m)):
                qu = jnp.where(rowc == DH + r, piece, qu)
            qbuf[g] = qu
            return carry

        lax.fori_loop(1, NB * U + 1, true_max, 0)

    def tcols(c):
        return (c // CPB, slice(None), slice(c % CPB * CK, (c % CPB + 1) * CK))

    def probs(u, c):
        return _bf16(pbuf[u, c * CK // 2:(c + 1) * CK // 2])

    def weighted_values(u, c):
        return _dot(vt[tcols(c)], probs(u, c))

    def finish_o(u, acc):
        linv = 1.0 / acc[DH:DH + 1]
        o = acc * linv
        obuf[u] = jnp.where(rowc == DH, linv, o)
        omrg[aligned(u * 2 * DH, 2 * DH, 8)] = merge_pair(o)

    k_groups = [(kvtab, r) for r in range((NV - NF) // 8)] + [(ktab, r) for r in range(NF // 8)]
    v_groups = [(kvtab, (NV - NF) // 8 + r) for r in range(ND // 8)]

    def attention(schedule, vpu_keys, pairing, u0, count, g_fwd=None, g_bwd=None):
        ops = [(schedule[j], int(schedule[j + 1])) for j in range(0, len(schedule), 2)]
        slot = {i: u0 + i for i in range(count)}
        slot[-1] = (u0 + U - 1) % U
        ds = {} if g_bwd is None else {(-1, NCH - 1): carry_ds[...]}
        chain = [None, None]
        unwritten = []

        def wide_product(i, c, rows_ref, groups, w_ref, at):
            if c == 0:
                w = w_ref[at]
                for d, r in enumerate([*range(DH), HP - 1]):
                    row = jnp.broadcast_to(w[r:r + 1], (8, NC))
                    for t in range(NC // 128):
                        qrow[i % 2, t, 2 + d] = row[:, t * 128:(t + 1) * 128]
            n, pairs = vpu_keys[i * NCH + c], pairing[i * NCH + c]
            groups = groups[len(groups) - n // 8:]
            head = _dot(rows_ref[c * CK:(c + 1) * CK - n], w_ref[at])
            tiles = [[] for _ in groups]
            for t in range(NC // 128):
                shift = qrow[i % 2, t, 2 + DH]
                for tile, (tab, r) in zip(tiles, groups):
                    prev = chain.pop(0)
                    s = shift if prev is None else _after(u0, shift, prev)
                    blocks = [tab[c, r, d:d + 4] * qrow[i % 2, t, 2 + d:6 + d] for d in range(0, DH, 4)]
                    terms = [block[d] for block in blocks for d in range(4)]
                    for j in range(DH - pairs):
                        term = terms.pop(0)
                        if (j + 1) * pairs // (DH - pairs) > j * pairs // (DH - pairs):
                            term = term + terms.pop(0)
                        s = s + term
                    chain.append(s)
                    tile.append(s)
            return jnp.concatenate([head] + [jnp.concatenate(tile, axis=1) for tile in tiles], axis=0)

        def write_probs():
            for u, c, packed in unwritten:
                pbuf[u, c * CK // 2:(c + 1) * CK // 2] = packed
            unwritten.clear()

        def run(name, i, c):
            if name == "S":
                e = pltpu.bitcast(jnp.exp2(wide_product(i, c, kp, k_groups, qbuf, g_fwd + i + 1)), U32)
                parity = [jnp.concatenate([e[k:k + 8] for k in range(j, CK, 16)], axis=0) for j in (0, 8)]
                unwritten.append((slot[i], c, _interleave(*parity)))
            elif name == "D":
                if g_fwd is None:
                    dp = wide_product(i, c, vp, v_groups, dobuf, slot[i])
                else:
                    dp = _dot(vp[c * CK:(c + 1) * CK], dobuf[slot[i]])
                ds[i, c] = (probs(slot[i], c).astype(F32) * dp).astype(BF16)
            elif name == "V":
                dvt[tcols(c)] += _dot(dobuf[slot[i]], probs(slot[i], c), _NT)
            elif name == "K":
                dkt[tcols(c)] += _dot(qbuf[g_bwd + i + 1], ds[i, c], _NT)
            else:
                if name == "P":
                    if i >= 0:
                        write_probs()
                    total, acc = weighted_values(slot[i], c), carry_o
                else:
                    total, acc = _dot(kt[tcols(c)], ds[i, c]), carry_dq
                if c:
                    total = acc[...] + total
                if c < NCH - 1:
                    acc[...] = total
                elif name == "P":
                    finish_o(slot[i], total)
                else:
                    qbuf[g_bwd + i if i >= 0 else jnp.where(u0 > 0, g_bwd + i, g_bwd)] = total

        for step in range(count * NCH):
            for name, lag in ops:
                run(name, *divmod(step - lag, NCH))
        write_probs()
        if g_bwd is not None:
            carry_ds[...] = ds[count - 1, NCH - 1]

    def dense(b):
        ga, sb, cb1, gb = (mod(j) for j in (2, 3, 4, 5))
        tok = (slice(0, BQ // 2), slice(BQ // 2, BQ))

        def operands(y):
            y11, y12, y21, y22 = (y[k:k + KH, t] for k in (0, KH) for t in tok)
            return (_right_order(_left_terms(y11, y12, y21, y22)),
                    _right_order(_left_terms(y11, y21, y12, y22)), y[2 * KH:].astype(BF16))

        def expand(w, r, y):
            rest = [_dot(_bf16(wf_terms[w, 7, _half(r), k:k + 128]), y[2]) for k in (0, 128)]
            quads = _strassen([_bf16(wf_terms[w, m, _half(r)]) for m in range(7)], y[0])
            return [quads[2 * i + j] + rest[i][:, tok[j]] for i in (0, 1) for j in (0, 1)]

        def outer(terms, rows, y):
            rest = [_dot(t, y[2], _NT) for t in rows]
            quads = _strassen(terms, y[1], _NT)
            return [jnp.concatenate([quads[2 * i], quads[2 * i + 1], rest[i]], axis=1) for i in (0, 1)]

        def activate(r, pre, dact):
            du, act = [], []
            for uq, dq in zip(pre, dact):
                sig = 0.5 * jnp.tanh(0.5 * uq) + 0.5
                act.append(uq * sig)
                du.append(dq * (sig + act[-1] * (1.0 - sig)))
            for w, quads in enumerate((du, act)):
                for m, term in enumerate(_left_terms(*quads) + [t.astype(BF16) for t in quads[1:3]]):
                    ffn_terms[w, m, _half(r)] = _words(term)

        def hidden(w, m, r=slice(0, FH)):
            return _bf16(ffn_terms[w, m, _half(r)])

        def weight_grad(w, r, y):
            rows = [jnp.concatenate([hidden(w, m, r) for m in pair], axis=1) for pair in ((2, 7), (8, 3))]
            for i, half in enumerate(outer([hidden(w, m, r) for m in range(7)], rows, y)):
                dwf[w, i * FH + r.start:i * FH + r.stop] += half

        def contract(w):
            left = [jnp.concatenate([_bf16(wft_terms[w, m, j]) for j in range(FT)], axis=1)[:, :FH]
                    for m in range(7)]
            quads = _strassen(left, _right_order([hidden(w, m) for m in range(7)]))
            return jnp.concatenate([jnp.concatenate(quads[i:i + 2], axis=1) for i in (0, 2)], axis=0)

        chunks = [slice(r, r + FM) for r in range(0, FH, FM)]
        g = gs[block_rows(b)].T.astype(F32)
        df = operands(_paced(b, lambda r, one: g[r] * one * gb[r], jnp.ones((1, BQ), F32), D, 8))
        finish_o(U - 1, carry_o[...] + weighted_values(U - 1, NCH - 1))
        o = omrg[...]
        a = _dot(_bf16(side_by_side(wot)), o.astype(BF16))
        x1 = _bf16(xt[b]).astype(F32) + ga * a
        xc2, _, rstd2 = _center(b, x1)
        h2 = operands(_paced(b, lambda r, rs: xc2[r] * rs * cb1[r] + sb[r], rstd2, D, 32))
        for r, dact in zip(chunks, [expand(1, r, df) for r in chunks]):
            activate(r, expand(0, r, h2), dact)
        weight_grad(0, chunks[0], h2)
        dh2 = contract(0)
        dhx = dh2 * (xc2 * rstd2)
        dxh = dh2 * cb1
        m1, m2 = _row_mean(dxh), _row_mean(dhx * cb1) * rstd2
        d1 = _paced(b, lambda r, m: g[r] + rstd2 * (dxh[r] - xc2[r] * m - m1), m2, D, 160)
        dx1[b] = d1
        da = d1 * ga
        f = contract(1)
        do = _dot(wo[...], da.astype(BF16))
        halves = (o[:D // 2], o[D // 2:])
        terms = _left_terms(*[t[:, k] for t in halves for k in tok])
        dwo[...] += jnp.concatenate(outer(terms, [t.astype(BF16) for t in halves], operands(da)), axis=0)
        for i, r in enumerate(chunks):
            if i:
                weight_grad(0, r, h2)
            weight_grad(1, r, df)
        gs[block_rows(b)] = (x1 + gb * f).astype(BF16).T
        dmod[2] += _fold(d1 * a)
        dmod[3] += _fold(dh2)
        dmod[4] += _fold(dhx)
        dmod[5] += _fold(g * f)
        for u in range(U):
            ou = obuf[u]
            if u:
                ou = jnp.concatenate([ou[:16], _after(b, ou[16:], dos[16:])], axis=0)
            dos = jnp.where(rowc < DH, _round(split_pair(do, u) * ou[DH:DH + 1]), 0.0)
            delta = jnp.sum(dos * ou, axis=0, keepdims=True)
            hi = _round(delta)
            for r, piece in ((DH, hi), (DH + 1, _round(delta - hi)), (HP - 1, -delta)):
                dos = jnp.where(rowc == r, piece, dos)
            dobuf[u] = dos

    def forward_only(u, carry):
        @pl.when(u == 1)
        def _():
            cp_wm1.start()
            cp_g.start()

        attention(*SCHED_FWD, 2 * u, 2, g_fwd=2 * u)
        set_up(2 * u)
        set_up(2 * u + 1)
        return carry

    def set_up(u):
        column_table(kvtab, u, jnp.concatenate(
            [kp[aligned((u + 1) * CK - NV, NV - NF, 8)], vp[aligned((u + 1) * CK - ND, ND, 8)]], axis=0))
        w, j = u % 2, jnp.minimum(u // 2, FT - 1)
        top, low = wf[w, slab(j)], wf[w, aligned(FH + j * 128, 128, 16)]
        halves = (_words(top), _words(low))
        rest = jnp.concatenate([t[:, 2 * KH:] for t in halves], axis=1)
        for m, term in enumerate(_left_words(*[t[:, k:k + KH] for t in halves for k in (0, KH)]) + [rest]):
            wf_terms[w, m, aligned(j * 64, 64, 64)] = term
        halves = (_words(top.T), _words(low.T))
        for m, term in enumerate(_left_words(*[t[r:r + D // 4] for r in (0, D // 4) for t in halves])):
            wft_terms[w, m, j] = term
        j = jnp.minimum(u, D // 128 - 1)
        wot[j] = _words(wo[slab(j)].T)

    def block(b, carry):
        dense(b)

        @pl.when(b < NB - 1)
        def _():
            def merged(i, carry):
                u = i * 2
                attention(*SCHED_MERGED, u, 2, g_fwd=(b + 1) * U + u, g_bwd=b * U + u)
                return carry

            lax.fori_loop(0, U // 2, merged, 0)

        return carry

    def token_sums(j):
        drow[j] = jnp.broadcast_to(jnp.sum(dmod[j].T, axis=0, keepdims=True), (8, D))

    def backward_only(u, carry):
        attention(*SCHED_BWD, 2 * u, 2, g_bwd=(NB - 1) * U + 2 * u)
        wf[:, share(u, FF)] = dwf[:, share(u, FF)].astype(BF16)
        token_sums(2 + u % 4)
        wo[share(u, D)] = dwo[share(u, D)].astype(BF16)
        return carry

    cp_wo.wait()
    cp_w1.wait()
    cp_w2.wait()
    lax.fori_loop(0, U // 2, forward_only, 0)
    carry_o[...] += weighted_values(U - 1, NCH - 3) + weighted_values(U - 1, NCH - 2)
    cp_wm1.wait()
    cp_g.wait()
    for j in range(2, 6):
        modulation(j)
    lax.fori_loop(0, NB, block, 0)
    stores = [cout(0, gs, out_hbm), cout(1, wf.at[0, pl.ds(0, FF)], gw1t_hbm),
              cout(2, wf.at[1, pl.ds(0, FF)], gw2_hbm), cout(3, wo, gwo_hbm)]
    stores[0].start()
    lax.fori_loop(0, U // 2, backward_only, 0)
    for cp in stores[1:]:
        cp.start()
    dkt[tcols(NCH - 1)] += _dot(qbuf[NB * U], carry_ds[...], _NT)
    qbuf[NB * U - 1] = carry_dq[...] + _dot(kt[tcols(NCH - 1)], carry_ds[...])

    def modulation_grad(seed, start, count, parts):
        totals, prev = [], None
        for i in range(0, count, 16):
            rows = aligned(start + i, 16, 16)
            total = None
            for j, t in ((j, t) for j in parts for t in range(0, D, 128)):
                cols = slice(j * D + t, j * D + t + 128)
                grad = drow[j, :, t:t + 128]
                if prev is not None:
                    grad = _after(seed, grad, prev)
                grad = jnp.concatenate([grad, grad], axis=0)
                part = wm[rows, cols].astype(F32) * grad
                total = part if total is None else total + part
                gw = sct[rows] * grad
                wm[rows, cols] = gw.astype(BF16)
                prev = gw[8:] + part[8:]
            totals.append(total)
        return jnp.concatenate(totals, axis=0)

    def input_grad(b, carry):
        dkv = jnp.concatenate(
            [jnp.where(rowb < DH, dkt[b] * scale, 0.0), jnp.where(rowb < DH, dvt[b], 0.0)], axis=0).astype(BF16)
        dq = jnp.concatenate([merge_pair(qbuf[b * U + u]) for u in range(U)], axis=0).astype(BF16)
        dq_rest[b] = dq[QE:]
        dh = _dot(_bf16(wqkv[:, D:D + KV]), dkv) + _dot(_bf16(wqkv[:, :D]), dq)
        dwo[0:KV + QE] += _dot(jnp.concatenate([dkv, dq[:QE]], axis=0), _bf16(ht[b]), _NT)
        rstd = stats[b, 1:2]
        xh = (_bf16(xt[b]).astype(F32) - stats[b, 0:1]) * rstd
        dmod[0] += _fold(dh)
        dmod[1] += _fold(dh * xh)
        dxh = dh * mod(1)
        m1, m2 = _row_mean(dxh), _row_mean(dxh * xh)
        d0 = _paced(b, lambda r, m: dx1[b, r] + rstd * (dxh[r] - xh[r] * m - m1), m2, D, 16)
        xs[block_rows(b)] = d0.astype(BF16).T
        cout(4, xs.at[block_rows(b)], dx_hbm.at[block_rows(b)]).start()
        rows = aligned(b * (D // NB), D // NB, 16)
        gc_col[rows] = modulation_grad(b, b * (D // NB), D // NB, (2, 3, 4, 5))
        cout(5, wm.at[rows, other_cols], gwm_hbm.at[rows, other_cols]).start()
        return carry + 1

    def query_weight_grad(i):
        dq = jnp.concatenate([dq_rest[b, slab(i)] for b in range(NB)], axis=1)
        wq[:, slab(QE // 128 + i)] = _dot(dq, _bf16(side_by_side(ht)), _NT).astype(BF16).T

    dwo[0:KV + QE] = jnp.zeros((KV + QE, D), F32)
    blocks_done = lax.fori_loop(0, NB, input_grad, 0)
    stores += [cout(4, xs, dx_hbm), cout(5, wm.at[:, other_cols], gwm_hbm.at[:, other_cols])]
    token_sums(0)
    token_sums(1)
    query_weight_grad(0)
    gc_col[...] += modulation_grad(blocks_done, 0, D, (0, 1))
    gsc = jnp.sum(gc_col[...].T, axis=0, keepdims=True)
    cb[...] = (gsc * c_sig * (1.0 + cf * (1.0 - c_sig))).astype(BF16)
    wkt[...] = dwo[0:DH].astype(BF16)
    wvt[...] = dwo[HP:HP + DH].astype(BF16)
    wq[:, 0:QE] = dwo[KV:KV + QE].astype(BF16).T
    head, last = pl.ds(0, QE + 128), pl.ds(QE + 128, D - QE - 128)
    late = [cout(6, wm.at[:, norm1_cols], gwm_hbm.at[:, norm1_cols]), cout(7, cb, gc_hbm),
            cout(8, wkt, gwkt_hbm), cout(9, wvt, gwvt_hbm), cout(10, wq.at[:, head], gwq_hbm.at[:, head])]
    for cp in late:
        cp.start()

    def last_slabs(i, carry):
        query_weight_grad(i)
        cols = slab(QE // 128 + i)
        cout(11, wq.at[:, cols], gwq_hbm.at[:, cols]).start()
        return carry

    lax.fori_loop(1, (D - QE) // 128, last_slabs, 0)
    late.append(cout(11, wq.at[:, last], gwq_hbm.at[:, last]))
    for cp in stores + late:
        cp.wait()


@jax.jit
def pallas_adaLN_cond__grouped_kv_mqa__dense_activation_silu__prompt_kernel(
    A_x: jax.Array,
    A_wq: jax.Array,
    A_wk: jax.Array,
    A_wv: jax.Array,
    A_wo: jax.Array,
    B_x: jax.Array,
    B_w1: jax.Array,
    B_w2: jax.Array,
    c: jax.Array,
    w_mod: jax.Array,
    grad_out: jax.Array,
):
    del B_x
    _, S, D = A_x.shape
    FF = B_w1.shape[1]
    DH = D // HEADS
    NB = S // BQ
    U = HEADS // 2
    FT = pl.cdiv(FF // 2, 128)
    vmem = pltpu.VMEM

    def sds(*shape):
        return jax.ShapeDtypeStruct(shape, BF16)

    scratch = dict(
        pbuf=vmem((U, S // 2, NC), U32),
        carry_o=vmem((HP, NC), F32), carry_dq=vmem((HP, NC), F32), carry_ds=vmem((CK, NC), BF16),
        obuf=vmem((U, HP, NC), F32), omrg=vmem((D, BQ), F32), dobuf=vmem((U, HP, NC), F32),
        qbuf=vmem((NB * U + 1, HP, NC), F32), kp=vmem((S, HP), F32), vp=vmem((S, HP), F32),
        kt=vmem((NB, HP, BQ), F32), vt=vmem((NB, HP, BQ), F32),
        dkt=vmem((NB, HP, BQ), F32), dvt=vmem((NB, HP, BQ), F32),
        ktab=vmem((S // CK, NF // 8, DH + 1, 8, 128), F32),
        kvtab=vmem((S // CK, (NV - NF + ND) // 8, DH + 1, 8, 128), F32),
        qrow=vmem((2, NC // 128, HP, 8, 128), F32),
        xs=vmem((S, D), BF16), gs=vmem((S, D), BF16), wq=vmem((D, D), BF16), wo=vmem((D, D), BF16),
        wf=vmem((2, 2 * FT * 128, D), BF16), wm=vmem((D, 6 * D), BF16),
        wqkv=vmem((D // 2, D + 128), U32), wot=vmem((D // 128, D // 2, 128), U32),
        wf_terms=vmem((2, 8, FT * 64, KH), U32), wft_terms=vmem((2, 7, FT, D // 4, 128), U32),
        xt=vmem((NB, D // 2, BQ), U32), ht=vmem((NB, D // 2, BQ), U32), dx1=vmem((NB, D, BQ), F32),
        dq_rest=vmem((NB, 384, BQ), BF16), stats=vmem((NB, 8, BQ), F32),
        modc=vmem((6, D, 128), F32), sct=vmem((D, 128), F32), dmod=vmem((6, D, 128), F32),
        gc_col=vmem((D, 128), F32), dwf=vmem((2, FF, D), F32), dwo=vmem((D, D), F32),
        ffn_terms=vmem((2, 9, FF // 4, BQ // 2), U32),
        wqkv_t=vmem((D // 2 + 32, D), U32), drow=vmem((8, 8, D), F32),
        wkt=vmem((DH, D), BF16), wvt=vmem((DH, D), BF16), cb=vmem((1, D), BF16),
        sem_in=pltpu.SemaphoreType.DMA((10 + NB,)), sem_out=pltpu.SemaphoreType.DMA((12,)),
    )
    hbm = pl.BlockSpec(memory_space=pl.ANY)
    out, dx, gwq, gwkt, gwvt, gwo, gw1t, gw2, gc, gwm = pl.pallas_call(
        _kernel,
        in_specs=[hbm] * 10,
        out_specs=[hbm] * 10,
        out_shape=[sds(S, D), sds(S, D), sds(D, D), sds(DH, D), sds(DH, D), sds(D, D),
                   sds(FF, D), sds(FF, D), sds(1, D), sds(D, 6 * D)],
        scratch_shapes=scratch,
        compiler_params=pltpu.CompilerParams(vmem_limit_bytes=127 * 1024 * 1024),
    )(A_x.reshape(S, D), A_wq, A_wk.T, A_wv.T, A_wo, B_w1.T, B_w2, c, w_mod, grad_out.reshape(S, D))
    return (out.reshape(1, S, D), dx.reshape(1, S, D), gwq, gwkt.T, gwvt.T, gwo, gw1t.T, gw2, gc, gwm)
```
